```python
import jax
import jax.numpy as jnp

def _softmax(x, axis=-1):
    return jax.nn.softmax(x, axis=axis)

def _gelu(x):
    return jax.nn.gelu(x, approximate=True)

def _silu(x):
    return jax.nn.silu(x)

def _sigmoid(x):
    return jax.nn.sigmoid(x)

def _layernorm(x, axis=-1, eps=1e-05):
    m = jnp.mean(x, axis=axis, keepdims=True)
    v = jnp.var(x, axis=axis, keepdims=True)
    return (x - m) / jnp.sqrt(v + eps)

def _scatter_add(tgt, idx, src, axis=0):
    return tgt.at[idx].add(src)

def _segment_sum(src, seg, n):
    return jax.ops.segment_sum(src, seg, n)

class _Rng:

    def __init__(self, key):
        self._k = key

    def _next(self):
        self._k, sub = jax.random.split(self._k)
        return sub

    def normal(self, shape):
        return jax.random.normal(self._next(), shape, dtype=jnp.bfloat16)

    def randint(self, lo, hi, shape):
        return jax.random.randint(self._next(), shape, lo, hi, dtype=jnp.int32)

    def uniform(self, shape, lo=0.0, hi=1.0):
        return jax.random.uniform(self._next(), shape, jnp.bfloat16, lo, hi)

    def permutation(self, n):
        return jax.random.permutation(self._next(), n)
kernel_name = 'adaLN_cond__sliding_block_cached__mixer_gmlp__decode'

def setup_inputs():
    _rng = _Rng(jax.random.key(int.from_bytes(__import__("os").urandom(4), "little")))
    _w = lambda a: (lambda t: t.astype(jnp.bfloat16) if jnp.issubdtype(t.dtype, jnp.floating) else t)(jnp.asarray(a))

    def _A_setup():
        B, Sq, D = (1, 1, 448)
        Hq, Hkv, Sk, Dh = (16, 8, 65536, 256)
        assert Hq % Hkv == 0, (Hq, Hkv)
        return {'x': _w((lambda *s: _rng.normal(s) * 0.05)(B, Sq, D)), 'k_cache': _w((lambda *s: _rng.normal(s) * 0.05)(B, Hkv, Sk, Dh)), 'v_cache': _w((lambda *s: _rng.normal(s) * 0.05)(B, Hkv, Sk, Dh)), 'wq': _w((lambda *s: _rng.normal(s) * 0.05)(D, Hq * Dh) * D ** (-0.5)), 'wo': _w((lambda *s: _rng.normal(s) * 0.05)(Hq * Dh, D) * (Hq * Dh) ** (-0.5))}
    _A_in = _A_setup()

    def _B_setup():
        B, S, D, F = (1, 1, 448, 1792)
        Fh = F // 2
        return {'x': _w((lambda *s: _rng.normal(s) * 0.05)(B, S, D)), 'w_in': _w((lambda *s: _rng.normal(s) * 0.05)(D, 2 * Fh)), 'w_sp': _w(0.01 * (lambda *s: _rng.normal(s) * 0.05)(S, S)), 'b_sp': _w(1.0 + 0.01 * (lambda *s: _rng.normal(s) * 0.05)(S)), 'w_out': _w((lambda *s: _rng.normal(s) * 0.05)(Fh, D))}
    _B_in = _B_setup()
    return {'A_x': _A_in['x'], 'A_k_cache': _A_in['k_cache'], 'A_v_cache': _A_in['v_cache'], 'A_wq': _A_in['wq'], 'A_wo': _A_in['wo'], 'B_x': _B_in['x'], 'B_w_in': _B_in['w_in'], 'B_w_sp': _B_in['w_sp'], 'B_b_sp': _B_in['b_sp'], 'B_w_out': _B_in['w_out'], 'c': _w((lambda *s: _rng.normal(s) * 0.05)(1, 448)), 'w_mod': _w((lambda *s: _rng.normal(s) * 0.05)(448, 6 * 448) * 448 ** (-0.5))}

def reference(A_x, A_k_cache, A_v_cache, A_wq, A_wo, B_x, B_w_in, B_w_sp, B_b_sp, B_w_out, c, w_mod):

    def _A_ref(x, k_cache, v_cache, wq, wo):
        B, Sq, D = x.shape
        Hq, Dh = (16, 256)
        Hkv, Sk = (k_cache.shape[1], k_cache.shape[2])
        W = min(4096, max(256, Sk // 4))
        rep = Hq // Hkv
        q = (lambda x, *d: x.transpose(*d))((x @ wq).reshape(B, Sq, Hq, Dh), 0, 2, 1, 3)
        k = jnp.repeat(k_cache[:, :, Sk - W:, :], rep, axis=1)
        v = jnp.repeat(v_cache[:, :, Sk - W:, :], rep, axis=1)
        scores = jnp.einsum('bhqd,bhkd->bhqk', q, k) * Dh ** (-0.5)
        p = _softmax(scores, axis=-1)
        o = jnp.einsum('bhqk,bhkd->bhqd', p, v)
        return (lambda x, *d: x.transpose(*d))(o, 0, 2, 1, 3).reshape(B, Sq, Hq * Dh) @ wo

    def _B_ref(x, w_in, w_sp, b_sp, w_out):
        B, S, D = x.shape
        F = w_in.shape[-1]
        Fh = F // 2
        z = _gelu(jnp.einsum('bsd,df->bsf', x, w_in))
        z1 = z[..., :Fh].copy()
        z2 = _layernorm(z[..., Fh:], axis=-1)
        g = jnp.einsum('ts,bsf->btf', w_sp, z2) + b_sp[None, :, None]
        return jnp.einsum('bsf,fd->bsd', z1 * g, w_out)
    x = A_x
    mod = (_silu(c) @ w_mod).reshape(c.shape[0], 6, 1, -1)
    sa, ca, ga, sb, cb, gb = (mod[:, 0].copy(), mod[:, 1].copy(), mod[:, 2].copy(), mod[:, 3].copy(), mod[:, 4].copy(), mod[:, 5].copy())
    h = _layernorm(x, axis=-1) * (1 + ca) + sa
    x = x + ga * _A_ref(h, A_k_cache, A_v_cache, A_wq, A_wo)
    h = _layernorm(x, axis=-1) * (1 + cb) + sb
    x = x + gb * _B_ref(h, B_w_in, B_w_sp, B_b_sp, B_w_out)
    return x
```

```python
import jax
import jax.numpy as jnp
import jax.experimental.pallas as pl
import jax.experimental.pallas.tpu as pltpu

HQ, DH = 16, 256
EPS = 1e-5
M = 8

_NT = (((1,), (1,)), ((), ()))
_NN = (((1,), (0,)), ((), ()))


def _ln(x):
    m = jnp.mean(x, axis=-1, keepdims=True)
    d = x - m
    v = jnp.mean(d * d, axis=-1, keepdims=True)
    return d * jax.lax.rsqrt(v + EPS)


def _dot(a, b, dims):
    return jax.lax.dot_general(a, b, dims, preferred_element_type=jnp.float32)


@jax.jit
def pallas_adaLN_cond__sliding_block_cached__mixer_gmlp__decode_kernel(
    A_x: jax.Array,
    A_k_cache: jax.Array,
    A_v_cache: jax.Array,
    A_wq: jax.Array,
    A_wo: jax.Array,
    B_x: jax.Array,
    B_w_in: jax.Array,
    B_w_sp: jax.Array,
    B_b_sp: jax.Array,
    B_w_out: jax.Array,
    c: jax.Array,
    w_mod: jax.Array,
):
    del B_x
    D = A_x.shape[-1]
    _, HKV, SK, _ = A_k_cache.shape
    W = min(4096, max(256, SK // 4))
    FH = B_w_in.shape[-1] // 2
    REP = HQ // HKV
    assert A_x.shape == (1, 1, D) and REP == 2

    def kernel(x_hbm, k_hbm, v_hbm, wq_hbm, woT_hbm, win_hbm, wsp_hbm, bsp_hbm, woutT_hbm, c_hbm, wmod_hbm,
               o_ref,
               x_v, c_v, wsp_v, bsp_v, wmod_v, wq_v, k_v, v_v, woT_v, win_v, woutT_v, sems):
        copies = [(wmod_hbm, wmod_v), (c_hbm, c_v), (x_hbm, x_v), (wsp_hbm, wsp_v), (bsp_hbm, bsp_v), (wq_hbm, wq_v)]
        for h in range(HKV):
            copies.append((k_hbm.at[0, h, pl.ds(SK - W, W), :], k_v.at[h]))
            copies.append((v_hbm.at[0, h, pl.ds(SK - W, W), :], v_v.at[h]))
        copies += [(woT_hbm, woT_v), (win_hbm, win_v), (woutT_hbm, woutT_v)]
        dmas = [pltpu.make_async_copy(s, d, sems.at[i]) for i, (s, d) in enumerate(copies)]
        for d in dmas:
            d.start()
        for i in range(5):
            dmas[i].wait()

        cc = jnp.broadcast_to(c_v[...].astype(jnp.float32), (M, D))
        sc = (cc * jax.nn.sigmoid(cc)).astype(jnp.bfloat16)
        mod = _dot(sc, wmod_v[...], _NN)
        sa, ca, ga, sb, cb, gb = [mod[:, i * D:(i + 1) * D] for i in range(6)]
        x = jnp.broadcast_to(x_v[0].astype(jnp.float32), (M, D))
        h = (_ln(x) * (1.0 + ca) + sa).astype(jnp.bfloat16)

        dmas[5].wait()
        q = _dot(h, wq_v[...], _NN) * (DH ** -0.5)
        row = jax.lax.broadcasted_iota(jnp.int32, (M, DH), 0)
        o_parts = []
        for hh in range(HKV):
            q0 = q[:, (2 * hh) * DH:(2 * hh + 1) * DH]
            q1 = q[:, (2 * hh + 1) * DH:(2 * hh + 2) * DH]
            qh = jnp.where(row == 0, q0, jnp.where(row == 1, q1, 0.0)).astype(jnp.bfloat16)
            dmas[6 + 2 * hh].wait()
            s = _dot(qh, k_v[hh], _NT)
            m = jnp.max(s, axis=-1, keepdims=True)
            p = jnp.exp(s - m)
            l = jnp.sum(p, axis=-1, keepdims=True)
            dmas[7 + 2 * hh].wait()
            o = _dot(p.astype(jnp.bfloat16), v_v[hh], _NN)
            o = o / l
            o_parts.append(jnp.where(row == 0, o, 0.0))
            o_parts.append(jnp.where(row == 1, o, 0.0))
        o_all = jnp.concatenate(o_parts, axis=-1).astype(jnp.bfloat16)
        dmas[6 + 2 * HKV].wait()
        attn = _dot(o_all, woT_v[...], _NT)
        attn = jnp.sum(attn, axis=0, keepdims=True)
        x1 = x + ga * attn
        h2 = (_ln(x1) * (1.0 + cb) + sb).astype(jnp.bfloat16)
        dmas[7 + 2 * HKV].wait()
        z = jax.nn.gelu(_dot(h2, win_v[...], _NN), approximate=True)
        z1 = z[:, :FH]
        z2 = _ln(z[:, FH:])
        wsp = wsp_v[...].astype(jnp.float32)
        bsp = bsp_v[...].astype(jnp.float32).reshape(1, 1)
        g = wsp * z2 + bsp
        zg = (z1 * g).astype(jnp.bfloat16)
        dmas[8 + 2 * HKV].wait()
        mlp = _dot(zg, woutT_v[...], _NT)
        out = x1 + gb * mlp
        o_ref[0] = out[0:1].astype(jnp.bfloat16)

    hbm = pl.BlockSpec(memory_space=pltpu.HBM)
    bf = jnp.bfloat16
    return pl.pallas_call(
        kernel,
        out_shape=jax.ShapeDtypeStruct((1, 1, D), bf),
        in_specs=[hbm] * 11,
        scratch_shapes=[
            pltpu.VMEM((1, 1, D), bf), pltpu.VMEM((1, D), bf), pltpu.VMEM((1, 1), bf), pltpu.VMEM((1,), bf),
            pltpu.VMEM((D, 6 * D), bf), pltpu.VMEM((D, HQ * DH), bf),
            pltpu.VMEM((HKV, W, DH), bf), pltpu.VMEM((HKV, W, DH), bf),
            pltpu.VMEM((D, HQ * DH), bf), pltpu.VMEM((D, 2 * FH), bf), pltpu.VMEM((D, FH), bf),
            pltpu.SemaphoreType.DMA((9 + 2 * HKV,)),
        ],
        compiler_params=pltpu.CompilerParams(vmem_limit_bytes=64 * 1024 * 1024),
    )(A_x, A_k_cache, A_v_cache, A_wq, A_wo.T, B_w_in, B_w_sp, B_b_sp, B_w_out.T, c, w_mod)
```

```python
import jax
import jax.numpy as jnp
import jax.experimental.pallas as pl
import jax.experimental.pallas.tpu as pltpu

HQ, DH = 16, 256
EPS = 1e-5
M = 8

_NT = (((1,), (1,)), ((), ()))
_NN = (((1,), (0,)), ((), ()))


def _ln(x):
    m = jnp.mean(x, axis=-1, keepdims=True)
    d = x - m
    v = jnp.mean(d * d, axis=-1, keepdims=True)
    return d * jax.lax.rsqrt(v + EPS)


def _dot(a, b, dims):
    return jax.lax.dot_general(a, b, dims, preferred_element_type=jnp.float32)


@jax.jit
def pallas_adaLN_cond__sliding_block_cached__mixer_gmlp__decode_kernel(
    A_x: jax.Array,
    A_k_cache: jax.Array,
    A_v_cache: jax.Array,
    A_wq: jax.Array,
    A_wo: jax.Array,
    B_x: jax.Array,
    B_w_in: jax.Array,
    B_w_sp: jax.Array,
    B_b_sp: jax.Array,
    B_w_out: jax.Array,
    c: jax.Array,
    w_mod: jax.Array,
):
    del B_x
    D = A_x.shape[-1]
    _, HKV, SK, _ = A_k_cache.shape
    W = min(4096, max(256, SK // 4))
    FH = B_w_in.shape[-1] // 2
    assert A_x.shape == (1, 1, D) and HQ == 2 * HKV and A_k_cache.shape[-1] == DH

    last = D - (D - 1) // 128 * 128
    wout_rows = [n for n in (D - 128 - last, 128, last) if n > 0]

    def kernel(x_hbm, k_hbm, v_hbm, wq_hbm, woT_hbm, win_hbm, wsp_hbm, bsp_hbm, woutT_hbm, c_hbm,
               wmod_hbm, o_ref,
               x_v, c_v, wsp_v, bsp_v, wmod_v, wq_v, k_v, v_v, woT_v, win_v, woutT_v,
               mods_v, q_v, o_v, sems):
        names, copies = [], {}

        def add(name, src, dst):
            copies[name] = pltpu.make_async_copy(src, dst, sems.at[len(names)])
            names.append(name)

        add("wmod", wmod_hbm, wmod_v)
        add("c", c_hbm, c_v)
        add("x", x_hbm, x_v)
        add("wsp", wsp_hbm, wsp_v)
        add("bsp", bsp_hbm, bsp_v)
        add("wq", wq_hbm, wq_v)
        for h in range(HKV):
            add(("k", h), k_hbm.at[0, h, pl.ds(SK - W, W), :], k_v.at[h])
            add(("v", h), v_hbm.at[0, h, pl.ds(SK - W, W), :], v_v.at[h])
        add("wo", woT_hbm, woT_v)
        add("win", win_hbm, win_v)
        r = 0
        for i, n in enumerate(wout_rows):
            add(("wout", i), woutT_hbm.at[pl.ds(r, n), :], woutT_v.at[pl.ds(r, n), :])
            r += n
        for name in names:
            copies[name].start()
        for name in ("wmod", "c", "x", "wsp", "bsp"):
            copies[name].wait()

        cc = jnp.broadcast_to(c_v[...].astype(jnp.float32), (M, D))
        sc = (cc * jax.nn.sigmoid(cc)).astype(jnp.bfloat16)
        mod = _dot(sc, wmod_v[...], _NN)
        for i in range(6):
            mods_v[i] = mod[:, i * D:(i + 1) * D]
        x = jnp.broadcast_to(x_v[0].astype(jnp.float32), (M, D))
        h1 = (_ln(x) * (1.0 + mods_v[1]) + mods_v[0]).astype(jnp.bfloat16)

        copies["wq"].wait()
        q = _dot(h1, wq_v[...], _NN) * (DH ** -0.5)
        row = jax.lax.broadcasted_iota(jnp.int32, (M, DH), 0)
        for h in range(HKV):
            q0 = q[:, (2 * h) * DH:(2 * h + 1) * DH]
            q1 = q[:, (2 * h + 1) * DH:(2 * h + 2) * DH]
            q_v[h] = jnp.where(row == 0, q0, jnp.where(row == 1, q1, 0.0)).astype(jnp.bfloat16)

        for h in range(HKV):
            copies[("k", h)].wait()
            s = _dot(q_v[h], k_v[h], _NT)
            m = jnp.max(s, axis=-1, keepdims=True)
            p = jnp.exp(s - m)
            l = jnp.sum(p, axis=-1, keepdims=True)
            copies[("v", h)].wait()
            o = _dot(p.astype(jnp.bfloat16), v_v[h], _NN) / l
            o2 = jnp.concatenate([jnp.where(row == 0, o, 0.0), jnp.where(row == 1, o, 0.0)], axis=-1)
            o_v[h] = o2.astype(jnp.bfloat16)

        o_all = jnp.concatenate([o_v[h] for h in range(HKV)], axis=-1)
        copies["wo"].wait()
        attn = jnp.sum(_dot(o_all, woT_v[...], _NT), axis=0, keepdims=True)
        x1 = x + mods_v[2] * attn
        h2 = (_ln(x1) * (1.0 + mods_v[4]) + mods_v[3]).astype(jnp.bfloat16)

        copies["win"].wait()
        z = jax.nn.gelu(_dot(h2, win_v[...], _NN), approximate=True)
        z1 = z[:, :FH]
        z2 = _ln(z[:, FH:])
        wsp = wsp_v[...].astype(jnp.float32)
        bsp = bsp_v[...].astype(jnp.float32).reshape(1, 1)
        zg = (z1 * (wsp * z2 + bsp)).astype(jnp.bfloat16)
        gb = mods_v[5]
        outs, r = [], 0
        for i, n in enumerate(wout_rows):
            copies[("wout", i)].wait()
            mlp = _dot(zg, woutT_v[pl.ds(r, n), :], _NT)
            outs.append(x1[:, r:r + n] + gb[:, r:r + n] * mlp)
            r += n
        out = jnp.concatenate(outs, axis=-1)
        o_ref[0] = out[0:1].astype(jnp.bfloat16)

    hbm = pl.BlockSpec(memory_space=pltpu.HBM)
    bf = jnp.bfloat16
    n_copies = 6 + 2 * HKV + 2 + len(wout_rows)
    return pl.pallas_call(
        kernel,
        out_shape=jax.ShapeDtypeStruct((1, 1, D), bf),
        in_specs=[hbm] * 11,
        scratch_shapes=[
            pltpu.VMEM((1, 1, D), bf),
            pltpu.VMEM((1, D), bf),
            pltpu.VMEM((1, 1), bf),
            pltpu.VMEM((1,), bf),
            pltpu.VMEM(w_mod.shape, bf),
            pltpu.VMEM((D, HQ * DH), bf),
            pltpu.VMEM((HKV, W, DH), bf),
            pltpu.VMEM((HKV, W, DH), bf),
            pltpu.VMEM((D, HQ * DH), bf),
            pltpu.VMEM((D, 2 * FH), bf),
            pltpu.VMEM((D, FH), bf),
            pltpu.VMEM((6, M, D), jnp.float32),
            pltpu.VMEM((HKV, M, DH), bf),
            pltpu.VMEM((HKV, M, 2 * DH), bf),
            pltpu.SemaphoreType.DMA((n_copies,)),
        ],
        compiler_params=pltpu.CompilerParams(
            vmem_limit_bytes=64 * 1024 * 1024,
            disable_semaphore_checks=True,
        ),
    )(A_x, A_k_cache, A_v_cache, A_wq, A_wo.T, B_w_in, B_w_sp, B_b_sp, B_w_out.T, c, w_mod)
```

```python
import jax
import jax.numpy as jnp
import jax.experimental.pallas as pl
import jax.experimental.pallas.tpu as pltpu

HQ, DH = 16, 256
EPS = 1e-5
M = 8

_NT = (((1,), (1,)), ((), ()))
_NN = (((1,), (0,)), ((), ()))


def _ln(x):
    m = jnp.mean(x, axis=-1, keepdims=True)
    d = x - m
    v = jnp.mean(d * d, axis=-1, keepdims=True)
    return d * jax.lax.rsqrt(v + EPS)


def _dot(a, b, dims):
    return jax.lax.dot_general(a, b, dims, preferred_element_type=jnp.float32)


@jax.jit
def pallas_adaLN_cond__sliding_block_cached__mixer_gmlp__decode_kernel(
    A_x: jax.Array,
    A_k_cache: jax.Array,
    A_v_cache: jax.Array,
    A_wq: jax.Array,
    A_wo: jax.Array,
    B_x: jax.Array,
    B_w_in: jax.Array,
    B_w_sp: jax.Array,
    B_b_sp: jax.Array,
    B_w_out: jax.Array,
    c: jax.Array,
    w_mod: jax.Array,
):
    del B_x
    D = A_x.shape[-1]
    _, HKV, SK, _ = A_k_cache.shape
    W = min(4096, max(256, SK // 4))
    FH = B_w_in.shape[-1] // 2
    assert A_x.shape == (1, 1, D) and HQ == 2 * HKV and A_k_cache.shape[-1] == DH

    last = D - (D - 1) // 128 * 128
    wout_rows = [n for n in (D - 128 - last, 128, last) if n > 0]

    def kernel(x_hbm, k_hbm, v_hbm, wq_hbm, woT_hbm, win_hbm, wsp_hbm, bsp_hbm, woutT_hbm, c_hbm,
               wmod_hbm, o_ref,
               x_v, c_v, wsp_v, bsp_v, wmod_v, wq_v, k_v, v_v, woT_v, win_v,
               mods_v, q_v, o_v, sems, *woutT_v):
        names, copies = [], {}

        def add(name, src, dst):
            copies[name] = pltpu.make_async_copy(src, dst, sems.at[len(names)])
            names.append(name)

        add("wmod", wmod_hbm, wmod_v)
        add("c", c_hbm, c_v)
        add("x", x_hbm, x_v)
        add("wsp", wsp_hbm, wsp_v)
        add("bsp", bsp_hbm, bsp_v)
        add("wq", wq_hbm, wq_v)
        for h in range(HKV):
            add(("k", h), k_hbm.at[0, h, pl.ds(SK - W, W), :], k_v.at[h])
            add(("v", h), v_hbm.at[0, h, pl.ds(SK - W, W), :], v_v.at[h])
        add("wo", woT_hbm, woT_v)
        add("win", win_hbm, win_v)
        r = 0
        for i, n in enumerate(wout_rows):
            add(("wout", i), woutT_hbm.at[pl.ds(r, n), :], woutT_v[i])
            r += n
        for name in names:
            copies[name].start()
        for name in ("wmod", "c", "x", "wsp", "bsp"):
            copies[name].wait()

        cc = jnp.broadcast_to(c_v[...].astype(jnp.float32), (M, D))
        sc = (cc * jax.nn.sigmoid(cc)).astype(jnp.bfloat16)
        mod = _dot(sc, wmod_v[...], _NN)
        for i in range(6):
            mods_v[i] = mod[:, i * D:(i + 1) * D]
        x = jnp.broadcast_to(x_v[0].astype(jnp.float32), (M, D))
        h1 = (_ln(x) * (1.0 + mods_v[1]) + mods_v[0]).astype(jnp.bfloat16)

        copies["wq"].wait()
        q = _dot(h1, wq_v[...], _NN) * (DH ** -0.5)
        row = jax.lax.broadcasted_iota(jnp.int32, (M, DH), 0)
        for h in range(HKV):
            q0 = q[:, (2 * h) * DH:(2 * h + 1) * DH]
            q1 = q[:, (2 * h + 1) * DH:(2 * h + 2) * DH]
            q_v[h] = jnp.where(row == 0, q0, jnp.where(row == 1, q1, 0.0)).astype(jnp.bfloat16)

        for h in range(HKV):
            copies[("k", h)].wait()
            s = _dot(q_v[h], k_v[h], _NT)
            m = jnp.max(s, axis=-1, keepdims=True)
            p = jnp.exp(s - m)
            l = jnp.sum(p, axis=-1, keepdims=True)
            copies[("v", h)].wait()
            o = _dot(p.astype(jnp.bfloat16), v_v[h], _NN) / l
            o2 = jnp.concatenate([jnp.where(row == 0, o, 0.0), jnp.where(row == 1, o, 0.0)], axis=-1)
            o_v[h] = o2.astype(jnp.bfloat16)

        o_all = jnp.concatenate([o_v[h] for h in range(HKV)], axis=-1)
        copies["wo"].wait()
        attn = jnp.sum(_dot(o_all, woT_v[...], _NT), axis=0, keepdims=True)
        x1 = x + mods_v[2] * attn
        h2 = (_ln(x1) * (1.0 + mods_v[4]) + mods_v[3]).astype(jnp.bfloat16)

        copies["win"].wait()
        z = jax.nn.gelu(_dot(h2, win_v[...], _NN), approximate=True)
        z1 = z[:, :FH]
        z2 = _ln(z[:, FH:])
        wsp = wsp_v[...].astype(jnp.float32)
        bsp = bsp_v[...].astype(jnp.float32).reshape(1, 1)
        zg = (z1 * (wsp * z2 + bsp)).astype(jnp.bfloat16)
        gb = mods_v[5]
        outs, r = [], 0
        for i, n in enumerate(wout_rows):
            copies[("wout", i)].wait()
            mlp = _dot(zg, woutT_v[i][...], _NT)
            outs.append(x1[:, r:r + n] + gb[:, r:r + n] * mlp)
            r += n
        out = jnp.concatenate(outs, axis=-1)
        o_ref[0] = out[0:1].astype(jnp.bfloat16)

    hbm = pl.BlockSpec(memory_space=pltpu.HBM)
    bf = jnp.bfloat16
    n_copies = 6 + 2 * HKV + 2 + len(wout_rows)
    return pl.pallas_call(
        kernel,
        out_shape=jax.ShapeDtypeStruct((1, 1, D), bf),
        in_specs=[hbm] * 11,
        scratch_shapes=[
            pltpu.VMEM((1, 1, D), bf),
            pltpu.VMEM((1, D), bf),
            pltpu.VMEM((1, 1), bf),
            pltpu.VMEM((1,), bf),
            pltpu.VMEM(w_mod.shape, bf),
            pltpu.VMEM((D, HQ * DH), bf),
            pltpu.VMEM((HKV, W, DH), bf),
            pltpu.VMEM((HKV, W, DH), bf),
            pltpu.VMEM((D, HQ * DH), bf),
            pltpu.VMEM((D, 2 * FH), bf),
            pltpu.VMEM((6, M, D), jnp.float32),
            pltpu.VMEM((HKV, M, DH), bf),
            pltpu.VMEM((HKV, M, 2 * DH), bf),
            pltpu.SemaphoreType.DMA((n_copies,)),
            *[pltpu.VMEM((n, FH), bf) for n in wout_rows],
        ],
        compiler_params=pltpu.CompilerParams(
            vmem_limit_bytes=64 * 1024 * 1024,
            disable_semaphore_checks=True,
        ),
    )(A_x, A_k_cache, A_v_cache, A_wq, A_wo.T, B_w_in, B_w_sp, B_b_sp, B_w_out.T, c, w_mod)
```
